```python
import os as _os
_os.environ.setdefault("JAX_PLATFORMS", "cpu")
import jax
import jax.numpy as jnp

def _softmax(x, axis=-1):
    return jax.nn.softmax(x, axis=axis)
def _gelu(x):
    return jax.nn.gelu(x, approximate=True)
def _silu(x):
    return jax.nn.silu(x)
def _sigmoid(x):
    return jax.nn.sigmoid(x)
def _layernorm(x, axis=-1, eps=1e-5):
    m = jnp.mean(x, axis=axis, keepdims=True)
    v = jnp.var(x, axis=axis, keepdims=True)
    return (x - m) / jnp.sqrt(v + eps)
def _scatter_add(tgt, idx, src, axis=0):
    return tgt.at[idx].add(src)
def _segment_sum(src, seg, n):
    return jax.ops.segment_sum(src, seg, n)
class _Rng:
    def __init__(self, key):
        self._k = key
    def _next(self):
        self._k, sub = jax.random.split(self._k)
        return sub
    def normal(self, shape):
        return jax.random.normal(self._next(), shape, dtype=jnp.bfloat16)
    def randint(self, lo, hi, shape):
        return jax.random.randint(self._next(), shape, lo, hi, dtype=jnp.int32)
    def uniform(self, shape, lo=0.0, hi=1.0):
        return jax.random.uniform(self._next(), shape, jnp.bfloat16, lo, hi)
    def permutation(self, n):
        return jax.random.permutation(self._next(), n)


kernel_name = 'sequential_preLN__sliding_local_dilated__mixer_s_mlp__prompt'

def setup_inputs():
    _rng = _Rng(jax.random.key(int.from_bytes(__import__("os").urandom(4), "little")))
    _w = (lambda a: (lambda t: t.astype(jnp.bfloat16) if jnp.issubdtype(t.dtype, jnp.floating) else t)(jnp.asarray(a)))
    def _A_setup():
        B, S, D = 1, 2048, 448
        return {
            "x": _w((lambda *s: _rng.normal(s) * 0.05)(B, S, D)),
            "wqkv": _w((lambda *s: _rng.normal(s) * 0.05)(D, 3 * D)),
            "wo": _w((lambda *s: _rng.normal(s) * 0.05)(D, D)),
        }
    _A_in = _A_setup()

    def _B_setup():
        B, S, D, F = 1, 2048, 448, 1792
        return {
            "x":  _w((lambda *s: _rng.normal(s) * 0.05)(B, S, D)),
            "w1": _w((lambda *s: _rng.normal(s) * 0.8)(D, D) * (D ** -0.5)),
            "w2": _w((lambda *s: _rng.normal(s) * 0.8)(D, D) * (D ** -0.5)),
            "w3": _w((lambda *s: _rng.normal(s) * 0.8)(D, F) * (D ** -0.5)),
            "w4": _w((lambda *s: _rng.normal(s) * 0.8)(F, D) * (F ** -0.5)),
        }
    _B_in = _B_setup()

    return {
        "A_x": _A_in["x"],
        "A_wqkv": _A_in["wqkv"],
        "A_wo": _A_in["wo"],
        "B_x": _B_in["x"],
        "B_w1": _B_in["w1"],
        "B_w2": _B_in["w2"],
        "B_w3": _B_in["w3"],
        "B_w4": _B_in["w4"],
    }

def reference(A_x, A_wqkv, A_wo, B_x, B_w1, B_w2, B_w3, B_w4):
    def _A_ref(x, wqkv, wo):
        B, S, D = x.shape
        H = 16; Dh = D // H
        W, dil = 8, 2
        qkv = (lambda x, *d: x.transpose(*d))((x @ wqkv).reshape(B, S, 3, H, Dh), 2, 0, 3, 1, 4)
        q, k, v = qkv[0], qkv[1], qkv[2]
        scale = Dh ** -0.5
        pos = jnp.arange(S)
        off = jnp.arange(W) * dil
        idx = pos[:, None] - off[None, :]
        mask = idx >= 0
        idx_c = jnp.where(mask, idx, 0).reshape(-1)
        kg = k[:, :, idx_c, :].reshape(B, H, S, W, Dh)
        vg = v[:, :, idx_c, :].reshape(B, H, S, W, Dh)
        logits = jnp.einsum("bhsd,bhswd->bhsw", q, kg) * scale
        logits = jnp.where(mask[None, None, :, :], logits, -1e9)
        attn = _softmax(logits, axis=-1)
        o = jnp.einsum("bhsw,bhswd->bhsd", attn, vg)
        return (lambda x, *d: x.transpose(*d))(o, 0, 2, 1, 3).reshape(B, S, D) @ wo

    def _B_ref(x, w1, w2, w3, w4):
        B, S, D = x.shape
        h = _gelu(_layernorm(x, axis=-1) @ w1)
        c = D // 4
        g0 = jnp.pad(h[:, :, 0*c:1*c], ((0, 0), (1, 0), (0, 0)))[:, :S, :]
        g1 = jnp.pad(h[:, :, 1*c:2*c], ((0, 0), (0, 1), (0, 0)))[:, 1:, :]
        g2 = jnp.pad(h[:, :, 2*c:3*c], ((0, 0), (2, 0), (0, 0)))[:, :S, :]
        g3 = jnp.pad(h[:, :, 3*c:   ], ((0, 0), (0, 2), (0, 0)))[:, 2:, :]
        hs = jnp.concatenate([g0, g1, g2, g3], axis=-1) @ w2
        x1 = x + hs
        h2 = _gelu(_layernorm(x1, axis=-1) @ w3) @ w4
        return x1 + h2

    x = A_x
    h = x + _A_ref(_layernorm(x, axis=-1), A_wqkv, A_wo)
    h2 = h + _B_ref(_layernorm(h, axis=-1), B_w1, B_w2, B_w3, B_w4)
    return h2
```

```python
import jax
import jax.numpy as jnp
from jax import lax
import jax.experimental.pallas as pl
import jax.experimental.pallas.tpu as pltpu

S = 2048
D = 448
F = 1792
H = 16
DH = D // H
W = 8
DIL = 2
L = 128
NT = S // L
TB = 2
NB = NT // TB
DW = D // 2
FH = F // 2
EPS = 1e-5
BF = jnp.bfloat16
F32 = jnp.float32
U32 = jnp.uint32

CFG_1 = ("q0 q1 k0 k1 v0 v1 o0 o1 w1_0 w1_1", 12, "KVKV")
CFG_2 = ("q0 q1 k0 k1 v0 v1 o0 o1 w1_0 w1_1", 9, "KVKV")
CFG_3 = ("q0 q1 k0 k1 v0 v1 w2_0 w2_1 o0 o1 w1_0 w1_1", 10, "KVKV")
CFG_S = ("w3a0 w3a1 q0 q1 k0 k1 v0 v1 w2_0 w2_1 o0 o1 w3b0 w3b1 w1_0 w1_1 w4_0 w4_1", None, "KVKV")
CFG_E = ("w3a0 w3a1 w2_0 w2_1 o0 o1 w3b0 w3b1 w1_0 w1_1 w4_0 w4_1", 9, "KVKV")
CFG_T = ("w3a0 w3a1 w2_0 w2_1 w3b0 w3b1 w4_0 w4_1", None, "KVKV")
CFG_L = ("w3a0 w3a1 w3b0 w3b1 w4_0 w4_1", None, "KVKV")


def _lo(w):
    return lax.bitcast_convert_type(w << 16, F32)


def _hi(w):
    return lax.bitcast_convert_type(w & jnp.uint32(0xFFFF0000), F32)


def _pk(a):
    return pltpu.bitcast(a, U32)


def _upk(a):
    return pltpu.bitcast(a, BF)


def _colsum(x):
    r = x.shape[0] // 8
    acc = [None] * 4
    for i in range(r):
        p = x[8 * i:8 * i + 8, :]
        acc[i % 4] = p if acc[i % 4] is None else acc[i % 4] + p
    return jnp.sum((acc[0] + acc[1]) + (acc[2] + acc[3]), axis=0, keepdims=True)


def _stats(parts):
    c = parts[0][0:1, :]
    d = jnp.concatenate([p - c for p in parts], axis=0)
    s1 = _colsum(d) * (1.0 / D)
    s2 = _colsum(d * d) * (1.0 / D)
    v = jnp.maximum(s2 - s1 * s1, 0.0)
    return c + s1, lax.rsqrt(v + EPS), v


def _gelu2(x):
    c = 0.7978845608028654
    return x + x * jnp.tanh(x * (c + (c * 0.044715) * (x * x)))


def _mm(a, b):
    return jnp.dot(_upk(a), b, preferred_element_type=F32)


class _Idx:
    def __init__(self, base, off):
        self.base, self.off = base, off


def _tiles(b):
    if isinstance(b, _Idx):
        return [b.base + (TB * b.off + j) for j in range(TB)]
    return [TB * b + j for j in range(TB)]


def _kernel(x_hbm, wqkv_hbm, wo_hbm, w1_hbm, w2_hbm, w3_hbm, w4_hbm, o_hbm,
            x_v, o_v, wqkv_n, wo_n, w1_n, w2_n, w3_n, w4_c,
            wqkv_t, wo_t, w1_t, w2_t, w3_t, wo32,
            q_s, k_s, v_s, h_s, y_s, g_s, n_s, r_s, x1_s,
            wsem, xsem, osem):
    def wcopy(i, src, dst):
        return pltpu.make_async_copy(src, dst, wsem.at[i])

    def xcopy(n):
        s = n if n < TB else min(n // TB + 1, 4)
        return pltpu.make_async_copy(x_hbm.at[:, n * L:(n + 1) * L], x_v.at[n],
                                     xsem.at[s])

    def ocopy(n):
        c = pl.multiple_of(n * L, L)
        return pltpu.make_async_copy(o_v.at[n], o_hbm.at[:, pl.ds(c, L)],
                                     osem.at[0])

    QC = (0, 512, 896, 3 * D)
    c_qkv = [wcopy(i, wqkv_hbm.at[:, QC[i]:QC[i + 1]],
                   wqkv_n.at[:, QC[i]:QC[i + 1]]) for i in range(3)]
    c_o = wcopy(3, wo_hbm, wo_n)
    c_1 = wcopy(3, w1_hbm, w1_n)
    c_2 = wcopy(4, w2_hbm, w2_n)
    c_3 = wcopy(5, w3_hbm, w3_n)
    c_4 = [wcopy(6, w4_hbm.at[:, j * L:(j + 1) * L], w4_c.at[j])
           for j in range(F // L)]

    xcopy(0).start()
    c_qkv[0].start()
    xcopy(1).start()
    c_qkv[1].start(priority=1)
    c_qkv[2].start(priority=1)
    for n in _tiles(1):
        xcopy(n).start(priority=1)
    c_o.start(priority=1)
    c_1.start(priority=1)

    w4_w = w4_c.bitcast(U32)
    x_w = x_v.bitcast(U32)
    k_w = k_s.bitcast(U32)
    v_w = v_s.bitcast(U32)
    g_w = g_s.bitcast(U32)
    n_w = n_s.bitcast(U32)

    zero_blk = jnp.zeros((D, L), BF)
    k_s[0] = zero_blk
    v_s[0] = zero_blk
    g_s[0] = zero_blk
    g_s[NT + 1] = zero_blk

    lane = lax.broadcasted_iota(jnp.int32, (8, L), 1)

    def ln1(n):
        xw = x_w[n]
        m, r, _ = _stats([_lo(xw), _hi(xw)])
        return ((x_v[n].astype(F32) - m) * r).astype(BF)

    def mq(n, xn):
        q_s[n] = _mm(wqkv_t[0:DW, :], xn)

    def mk(n, xn):
        k_s[n + 1] = _mm(wqkv_t[DW:2 * DW, :], xn).astype(BF)

    def mv(n, xn):
        v_s[n + 1] = _mm(wqkv_t[2 * DW:3 * DW, :], xn).astype(BF)

    def shifted(cur, prev, w):
        if w == 0:
            return cur
        return pltpu.roll(jnp.where(lane >= L - DIL * w, prev, cur), DIL * w, 1)

    def never():
        return k_w[0, 0:8, :] != 0

    def tie_rhs(rhs, tok):
        head = jnp.where(never(), lax.bitcast_convert_type(tok, U32),
                         _pk(rhs[0:16, :]))
        return jnp.concatenate([_upk(head), rhs[16:, :]], axis=0)

    def attn(n, toks, ahead, seq):
        nv = never()

        def tie(v):
            if ahead is None or len(toks) < ahead:
                return v
            return jnp.where(nv, lax.bitcast_convert_type(toks[-ahead], U32), v)

        def probs(half):
            acc = [None] * W
            for dp in range(DH // 2):
                r0 = half * 8 * DH + 2 * dp
                j0 = half * 8 * (DH // 2) + dp
                q0 = q_s[n, pl.ds(r0, 8, stride=DH), :]
                q1 = q_s[n, pl.ds(r0 + 1, 8, stride=DH), :]
                kc = k_w[n + 1, pl.ds(j0, 8, stride=DH // 2), :]
                kp = tie(k_w[n, pl.ds(j0, 8, stride=DH // 2), :])
                for w in range(W):
                    ks = shifted(kc, kp, w)
                    tt = q0 * _lo(ks) + q1 * _hi(ks)
                    acc[w] = tt if acc[w] is None else acc[w] + tt
                toks.append(acc[W - 1])
            lg = [a * (DH ** -0.5) for a in acc]
            if isinstance(n, int) and n == 0:
                lg = [jnp.where(lane >= DIL * w, lg[w], -1e9) for w in range(W)]
            m = lg[0]
            for w in range(1, W):
                m = jnp.maximum(m, lg[w])
            e = [jnp.exp(lw - m) for lw in lg]
            den = e[0]
            for w in range(1, W):
                den = den + e[w]
            rinv = 1.0 / den
            return [ew * rinv for ew in e]

        def mix(half, p):
            outs = []
            for dp in range(DH // 2):
                j0 = half * 8 * (DH // 2) + dp
                vc = v_w[n + 1, pl.ds(j0, 8, stride=DH // 2), :]
                vp = tie(v_w[n, pl.ds(j0, 8, stride=DH // 2), :])
                o0 = None
                o1 = None
                for w in range(W):
                    vs = shifted(vc, vp, w)
                    a0 = p[w] * _lo(vs)
                    a1 = p[w] * _hi(vs)
                    o0 = a0 if o0 is None else o0 + a0
                    o1 = a1 if o1 is None else o1 + a1
                toks.append(o1)
                outs.append(jnp.concatenate([o0, o1], axis=0).astype(BF))
            return outs

        if seq == "KVKV":
            per_half = [mix(h, probs(h)) for h in range(2)]
        else:
            ps = [probs(h) for h in range(2)]
            per_half = [mix(h, ps[h]) for h in range(2)]
        pieces = []
        for dp in range(DH // 2):
            pieces.append(per_half[0][dp])
            pieces.append(per_half[1][dp])
        return jnp.concatenate(pieces, axis=0)

    def mo(n, o):
        h = x_v[n].astype(F32) + _mm(wo_t[...], o)
        h_s[n] = h
        m, r, v = _stats([h])
        y_s[n, 0:8, :] = jnp.broadcast_to(m, (8, L))
        y_s[n, 8:16, :] = jnp.broadcast_to(r, (8, L))
        r2 = lax.rsqrt(v * r * r + EPS)
        return ((h_s[n] - m) * (r * r2)).astype(BF)

    def m1(n, z):
        g_s[n + 1] = (0.5 * _gelu2(_mm(w1_t[...], z))).astype(BF)

    C = DW // 4
    lane_c = lax.broadcasted_iota(jnp.int32, (C, L), 1)

    def from_prev(n, g, s):
        cur = g_w[n + 1, g * C:(g + 1) * C, :]
        prev = g_w[n, g * C:(g + 1) * C, :]
        return pltpu.roll(jnp.where(lane_c >= L - s, prev, cur), s, 1)

    def from_next(n, g, s):
        cur = g_w[n + 1, g * C:(g + 1) * C, :]
        nxt = g_w[n + 2, g * C:(g + 1) * C, :]
        return pltpu.roll(jnp.where(lane_c < s, nxt, cur), L - s, 1)

    def m2(n, j):
        g = _upk(jnp.concatenate(
            [from_prev(n, 0, 1), from_next(n, 1, 1),
             from_prev(n, 2, 2), from_next(n, 3, 2)], axis=0))
        h = h_s[n]
        y = (h - y_s[n, 0:1, :]) * y_s[n, 8:9, :]
        x1 = y + _mm(w2_t[...], g)
        x1_s[j] = x1
        r_s[n] = h + x1
        m, r, _ = _stats([x1])
        n_s[n] = ((x1_s[j] - m) * r).astype(BF)

    def m3(n, part):
        r0 = part * (FH // 2)
        return _gelu2(_mm(w3_t[r0:r0 + FH // 2, :], _upk(n_w[n]))).astype(BF)

    def m4(n, h3a, h3b):
        h3 = jnp.concatenate([h3a, h3b], axis=0)
        w4 = jnp.concatenate([w4_w[j] for j in range(F // L)], axis=1)
        o_v[n] = (r_s[n] + 0.5 * _mm(w4, h3)).astype(BF)

    def step(cfg, a=None, b=None, c1=None, c23=None, extra=None):
        order, ahead, seq = cfg
        ta, tb, tc1, tc23 = (None if v is None else _tiles(v)
                             for v in (a, b, c1, c23))
        xn, o, z, h3 = {}, {}, {}, {}
        if extra is not None:
            extra()
        toks = []
        for item in order.split():
            item, _, ms = item.partition("@")
            name, j = item[:-1], int(item[-1])
            if name in ("q", "k", "v"):
                if j not in xn:
                    xn[j] = ln1(ta[j])
                rhs = xn[j]
                if ms:
                    rhs = tie_rhs(rhs, toks[int(ms)])
                {"q": mq, "k": mk, "v": mv}[name](ta[j], rhs)
            elif name == "att":
                o[j] = attn(tb[j], toks, ahead, seq)
            elif name == "o":
                if j not in o:
                    o[j] = attn(tb[j], toks, ahead, seq)
                z[j] = mo(tb[j], o[j])
            elif name == "w1_":
                m1(tb[j], z[j])
            elif name == "w2_":
                m2(tc1[j], j)
            elif name in ("w3a", "w3b"):
                h3[name, j] = m3(tc23[j], int(name == "w3b"))
            elif name == "w4_":
                m4(tc23[j], h3["w3a", j], h3["w3b", j])
            else:
                raise ValueError(item)
        if c23 is not None:
            for n in tc23:
                ocopy(n).start()

    def prep_wo_w1():
        w32 = wo_n[...].astype(F32)
        for j in range(4):
            cw = min(L, D - j * L)
            wo32[j, :, 0:cw] = w32[:, j * L:j * L + cw]
        rows = []
        for dp in range(DH // 2):
            for half in range(2):
                for par in range(2):
                    r0 = half * 8 * DH + 2 * dp + par
                    rows.append(jnp.concatenate(
                        [wo32[j, pl.ds(r0, 8, stride=DH), 0:min(L, D - j * L)]
                         for j in range(4)], axis=1))
        wo_t[...] = _pk(jnp.concatenate(rows, axis=0).astype(BF).T)
        w1_t[...] = _pk(w1_n[...].T)

    def prep_w2():
        w2_t[...] = _pk(w2_n[...].T)

    def prep_w3():
        w3_t[...] = _pk(w3_n[...].T)

    def prep_qkv(i):
        wqkv_t[QC[i] // 2:QC[i + 1] // 2, :] = _pk(
            wqkv_n[:, QC[i]:QC[i + 1]].T)

    xcopy(0).wait()
    xn0 = ln1(0)
    c_qkv[0].wait()
    xcopy(1).wait()
    prep_qkv(0)
    xn1 = ln1(1)
    c_qkv[1].wait()
    prep_qkv(1)
    mq(0, xn0)
    mq(1, xn1)
    c_qkv[2].wait()
    c_2.start(priority=1)
    for n in _tiles(2):
        xcopy(n).start(priority=1)
    c_3.start(priority=1)
    prep_qkv(2)
    mk(0, xn0)
    mk(1, xn1)
    mv(0, xn0)
    mv(1, xn1)

    for n in _tiles(1):
        xcopy(n).wait()
    c_o.wait()
    c_1.wait()
    for n in range(3 * TB, NT):
        xcopy(n).start(priority=1)
    for c in c_4:
        c.start(priority=1)
    step(CFG_1, a=1, b=0, extra=prep_wo_w1)
    for n in _tiles(2):
        xcopy(n).wait()
    c_2.wait()
    step(CFG_2, a=2, b=1, extra=prep_w2)
    for n in range(3 * TB, NT):
        xcopy(n).wait()
    c_3.wait()
    step(CFG_3, a=3, b=2, c1=0, extra=prep_w3)
    for c in c_4:
        c.wait()

    def steady(s, carry):
        u = s * TB
        step(CFG_S, a=_Idx(u, 4), b=_Idx(u, 3), c1=_Idx(u, 1), c23=_Idx(u, 0))
        return carry

    lax.fori_loop(0, NB - 4, steady, 0)

    step(CFG_E, b=NB - 1, c1=NB - 3, c23=NB - 4)

    def tail(t, carry):
        u = t * TB
        step(CFG_T, c1=_Idx(u, 1), c23=_Idx(u, 0))
        return carry

    lax.fori_loop(NB - 3, NB - 1, tail, 0)
    step(CFG_L, c23=NB - 1)

    for n in range(NT):
        ocopy(n).wait()


@jax.jit
def pallas_sequential_preLN__sliding_local_dilated__mixer_s_mlp__prompt_kernel(
    A_x: jax.Array,
    A_wqkv: jax.Array,
    A_wo: jax.Array,
    B_x: jax.Array,
    B_w1: jax.Array,
    B_w2: jax.Array,
    B_w3: jax.Array,
    B_w4: jax.Array,
):
    del B_x
    xt = A_x.reshape(S, D).T
    hbm = pl.BlockSpec(memory_space=pltpu.HBM)
    out = pl.pallas_call(
        _kernel,
        out_shape=jax.ShapeDtypeStruct((D, S), BF),
        in_specs=[hbm] * 7,
        out_specs=hbm,
        scratch_shapes=[
            pltpu.VMEM((NT, D, L), BF),
            pltpu.VMEM((NT, D, L), BF),
            pltpu.VMEM((D, 3 * D), BF),
            pltpu.VMEM((D, D), BF),
            pltpu.VMEM((D, D), BF),
            pltpu.VMEM((D, D), BF),
            pltpu.VMEM((D, F), BF),
            pltpu.VMEM((F // L, D, L), BF),
            pltpu.VMEM((3 * DW, D), U32),
            pltpu.VMEM((DW, D), U32),
            pltpu.VMEM((DW, D), U32),
            pltpu.VMEM((DW, D), U32),
            pltpu.VMEM((FH, D), U32),
            pltpu.VMEM((4, D, L), F32),
            pltpu.VMEM((NT, D, L), F32),
            pltpu.VMEM((NT + 1, D, L), BF),
            pltpu.VMEM((NT + 1, D, L), BF),
            pltpu.VMEM((NT, D, L), F32),
            pltpu.VMEM((NT, 16, L), F32),
            pltpu.VMEM((NT + 2, D, L), BF),
            pltpu.VMEM((NT, D, L), BF),
            pltpu.VMEM((NT, D, L), F32),
            pltpu.VMEM((TB, D, L), F32),
            pltpu.SemaphoreType.DMA((7,)),
            pltpu.SemaphoreType.DMA((5,)),
            pltpu.SemaphoreType.DMA((1,)),
        ],
        compiler_params=pltpu.CompilerParams(
            vmem_limit_bytes=96 * 1024 * 1024),
    )(xt, A_wqkv, A_wo, B_w1, B_w2, B_w3, B_w4.T)
    return out.T.reshape(1, S, D)
```

```python
import jax
import jax.numpy as jnp
from jax import lax
import jax.experimental.pallas as pl
import jax.experimental.pallas.tpu as pltpu

S = 2048
D = 448
F = 1792
H = 16
DH = D // H
W = 8
DIL = 2
L = 128
NT = S // L
TB = 2
NB = NT // TB
DW = D // 2
FH = F // 2
EPS = 1e-5
LAST_TILE = 15
RS = 320
BF = jnp.bfloat16
F32 = jnp.float32
U32 = jnp.uint32

QC = (0, 256, 512, 896, 1344)
START = "x0 c0 x1 c1 x2:1 x3:1 c2:1 x45:1 c3:1 wo:1"
PROLOGUE = (
    "W:x0 l:0 "
    "W:c0 T:c0 "
    "W:x1 ql:0 ql:1 "
    "W:c1+x2 T:c1 ql:2 qh:0 qh:1 "
    "W:x3+c2 S:w1 S:w2 S:x67 T:c2 qh:2 q:3 k:0 k:1 "
    "W:c3+x45 S:w3 A:0 k:2 aK:0 k:3 aK:1 T:c3 v:1 l:5 v:0 "
    "W:wo S:w4 S:xr A:8 v:2 T:wo aV:0 aK:3 aV:1 v:3 q:4 q:5 o:0 k:5 aK:2 "
    "v:4 l:4 k:4 aV:3 o:1 v:5 aV:2 "
    "W:w1+w2+x67+w3 A:10 T:w1 o:2 w1:0 T:w3 o:3 w1:1 q:7 k:6 v:6 w1:3 w1:2 "
    "k:7 T:w2 q:6 w2:0 w2:1 aK:4 aV:4 o:4 a:5 o:5 v:7 "
    "W:w4+xr")
CFG_S = ("w3a1 q1 w3b1 w3b0 w1_0 w3a0 v1 w1_1 v0 w4_0 q0 w2_1 w4_1 w2_0 "
         "o0 o1 k0 k1",
         8, "KVKV")
CFG_E = ("w1_0 w3b1 w1_1 w3b0 w3a0 w3a1 w2_1 w2_0 o0 o1 w4_1 w4_0",
         12, "KVKV")
CFG_F = ("w3b1 w2_0 w1_0 w1_1 w3a0 w3b0 w3a1 w2_1 w4_0 w4_1",
         None, "KVKV")
CFG_T = ("w3a1 w2_0 w3b1 w4_1 w3a0 w3b0 w4_0 w2_1",
         None, "KVKV")
CFG_L = ("w3a0 w3b0 w3a1 w4_0 w3b1 w4_1",
         None, "KVKV")

_WAITS = [it[2:].split("+") for it in PROLOGUE.split() if it.startswith("W:")]
_SEM = {name: i for i, grp in enumerate(_WAITS) for name in grp}


def _lo(w):
    return lax.bitcast_convert_type(w << 16, F32)


def _hi(w):
    return lax.bitcast_convert_type(w & jnp.uint32(0xFFFF0000), F32)


def _pk(a):
    return pltpu.bitcast(a, U32)


def _upk(a):
    return pltpu.bitcast(a, BF)


def _colsum(x):
    r = x.shape[0] // 8
    acc = [None] * 4
    for i in range(r):
        p = x[8 * i:8 * i + 8, :]
        acc[i % 4] = p if acc[i % 4] is None else acc[i % 4] + p
    return jnp.sum((acc[0] + acc[1]) + (acc[2] + acc[3]), axis=0, keepdims=True)


def _stats(parts):
    c = parts[0][0:1, :]
    d = jnp.concatenate([p - c for p in parts], axis=0)
    s1 = _colsum(d) * (1.0 / D)
    s2 = _colsum(d * d) * (1.0 / D)
    v = jnp.maximum(s2 - s1 * s1, 0.0)
    return c + s1, lax.rsqrt(v + EPS), v


def _gelu2(x):
    c = 0.7978845608028654
    return x + x * jnp.tanh(x * (c + (c * 0.044715) * (x * x)))


def _mm(a, b):
    return jnp.dot(_upk(a), b, preferred_element_type=F32)


class _Idx:
    def __init__(self, base, off):
        self.base, self.off = base, off


def _tiles(b):
    if isinstance(b, _Idx):
        return [b.base + (TB * b.off + j) for j in range(TB)]
    return [TB * b + j for j in range(TB)]


def _kernel(x_hbm, wqkv_hbm, wo_hbm, w1_hbm, w2_hbm, w3_hbm, w4_hbm, o_hbm,
            x_v, o_v, wqkv_n, wo_n, w1_n, w2_n, w3_n, w4_c,
            wqkv_t, wo_t, w1_t, w2_t, w3_t, wo32,
            q_s, k_s, v_s, h_s, y_s, g_s, n_s, r_s, x1_s, z_s,
            isem, osem):
    def icopy(name, src, dst):
        return pltpu.make_async_copy(src, dst, isem.at[_SEM[name]])

    def xcopies(name, tiles):
        return [icopy(name, x_hbm.at[:, n * L:(n + 1) * L], x_v.at[n])
                for n in tiles]

    def ocopy(n, r0=0, r1=D):
        c = pl.multiple_of(n * L, L)
        return pltpu.make_async_copy(o_v.at[n, r0:r1],
                                     o_hbm.at[r0:r1, pl.ds(c, L)], osem.at[0])

    dma = {"c%d" % i: [icopy("c%d" % i, wqkv_hbm.at[:, QC[i]:QC[i + 1]],
                             wqkv_n.at[:, QC[i]:QC[i + 1]])] for i in range(4)}
    dma.update({"x%d" % n: xcopies("x%d" % n, [n]) for n in range(4)})
    dma.update(x45=xcopies("x45", [4, 5]), x67=xcopies("x67", [6, 7]),
               xr=xcopies("xr", range(8, NT)),
               wo=[icopy("wo", wo_hbm, wo_n)], w1=[icopy("w1", w1_hbm, w1_n)],
               w2=[icopy("w2", w2_hbm, w2_n)], w3=[icopy("w3", w3_hbm, w3_n)],
               w4=[icopy("w4", w4_hbm.at[:, j * L:(j + 1) * L], w4_c.at[j])
                   for j in range(F // L)])
    for item in START.split():
        name, _, prio = item.partition(":")
        for c in dma[name]:
            c.start(priority=int(prio or 0))

    w4_w = w4_c.bitcast(U32)
    k_w = k_s.bitcast(U32)
    v_w = v_s.bitcast(U32)
    g_w = g_s.bitcast(U32)
    n_w = n_s.bitcast(U32)
    z_w = z_s.bitcast(U32)

    zero_blk = jnp.zeros((D, L), BF)
    k_s[0] = zero_blk
    v_s[0] = zero_blk
    g_s[0] = zero_blk
    g_s[NT + 1] = zero_blk

    lane = lax.broadcasted_iota(jnp.int32, (8, L), 1)

    def ln1(n):
        m, r, _ = _stats([x_v[n, 0:DW, :].astype(F32),
                          x_v[n, DW:D, :].astype(F32)])
        return ((x_v[n].astype(F32) - m) * r).astype(BF)

    def mq(n, xn, r0=0, r1=D):
        q_s[n, r0:r1, :] = _mm(wqkv_t[r0 // 2:r1 // 2, :], xn)

    def mk(n, xn):
        k_s[n + 1] = _mm(wqkv_t[DW:2 * DW, :], xn).astype(BF)

    def mv(n, xn):
        v_s[n + 1] = _mm(wqkv_t[2 * DW:3 * DW, :], xn).astype(BF)

    def shifted(cur, prev, w):
        if w == 0:
            return cur
        return pltpu.roll(jnp.where(lane >= L - DIL * w, prev, cur), DIL * w, 1)

    def tie(v, toks, ahead):
        if ahead is None or len(toks) < ahead:
            return v
        never = k_w[0, 0:8, :] != 0
        return jnp.where(never, lax.bitcast_convert_type(toks[-ahead], U32), v)

    def probs(n, half, toks, ahead):
        acc = [None] * W
        for dp in range(DH // 2):
            r0 = half * 8 * DH + 2 * dp
            j0 = half * 8 * (DH // 2) + dp
            q0 = q_s[n, pl.ds(r0, 8, stride=DH), :]
            q1 = q_s[n, pl.ds(r0 + 1, 8, stride=DH), :]
            kc = k_w[n + 1, pl.ds(j0, 8, stride=DH // 2), :]
            kp = tie(k_w[n, pl.ds(j0, 8, stride=DH // 2), :], toks, ahead)
            for w in range(W):
                ks = shifted(kc, kp, w)
                tt = q0 * _lo(ks) + q1 * _hi(ks)
                acc[w] = tt if acc[w] is None else acc[w] + tt
            toks.append(acc[W - 1])
        lg = [a * (DH ** -0.5) for a in acc]
        if isinstance(n, int) and n == 0:
            lg = [jnp.where(lane >= DIL * w, lg[w], -1e9) for w in range(W)]
        m = lg[0]
        for w in range(1, W):
            m = jnp.maximum(m, lg[w])
        e = [jnp.exp(lw - m) for lw in lg]
        den = e[0]
        for w in range(1, W):
            den = den + e[w]
        rinv = 1.0 / den
        return [ew * rinv for ew in e]

    def mix(n, half, p, toks, ahead):
        outs = []
        for dp in range(DH // 2):
            j0 = half * 8 * (DH // 2) + dp
            vc = v_w[n + 1, pl.ds(j0, 8, stride=DH // 2), :]
            vp = tie(v_w[n, pl.ds(j0, 8, stride=DH // 2), :], toks, ahead)
            o0 = None
            o1 = None
            for w in range(W):
                vs = shifted(vc, vp, w)
                a0 = p[w] * _lo(vs)
                a1 = p[w] * _hi(vs)
                o0 = a0 if o0 is None else o0 + a0
                o1 = a1 if o1 is None else o1 + a1
            toks.append(o1)
            outs.append(jnp.concatenate([o0, o1], axis=0).astype(BF))
        return outs

    def interleave(per_half):
        pieces = []
        for dp in range(DH // 2):
            pieces.append(per_half[0][dp])
            pieces.append(per_half[1][dp])
        return jnp.concatenate(pieces, axis=0)

    def attn(n, toks, ahead, seq):
        if seq == "KVKV":
            return interleave([mix(n, h, probs(n, h, toks, ahead), toks, ahead)
                               for h in range(2)])
        ps = [probs(n, h, toks, ahead) for h in range(2)]
        return interleave([mix(n, h, ps[h], toks, ahead) for h in range(2)])

    def mo(n, o):
        h = x_v[n].astype(F32) + _mm(wo_t[...], o)
        h_s[n] = h
        m, r, v = _stats([h])
        y_s[n, 0:8, :] = jnp.broadcast_to(m, (8, L))
        y_s[n, 8:16, :] = jnp.broadcast_to(r, (8, L))
        r2 = lax.rsqrt(v * r * r + EPS)
        z_s[n] = ((h_s[n] - m) * (r * r2)).astype(BF)

    def m1(n):
        g_s[n + 1] = (0.5 * _gelu2(_mm(w1_t[...], _upk(z_w[n])))).astype(BF)

    C = DW // 4
    lane_c = lax.broadcasted_iota(jnp.int32, (C, L), 1)

    def from_prev(n, g, s):
        cur = g_w[n + 1, g * C:(g + 1) * C, :]
        prev = g_w[n, g * C:(g + 1) * C, :]
        return pltpu.roll(jnp.where(lane_c >= L - s, prev, cur), s, 1)

    def from_next(n, g, s):
        cur = g_w[n + 1, g * C:(g + 1) * C, :]
        nxt = g_w[n + 2, g * C:(g + 1) * C, :]
        return pltpu.roll(jnp.where(lane_c < s, nxt, cur), L - s, 1)

    def m2(n, j):
        g = _upk(jnp.concatenate(
            [from_prev(n, 0, 1), from_next(n, 1, 1),
             from_prev(n, 2, 2), from_next(n, 3, 2)], axis=0))
        h = h_s[n]
        y = (h - y_s[n, 0:1, :]) * y_s[n, 8:9, :]
        x1 = y + _mm(w2_t[...], g)
        x1_s[j] = x1
        r_s[n] = h + x1
        m, r, _ = _stats([x1])
        n_s[n] = ((x1_s[j] - m) * r).astype(BF)

    def m3(n, part):
        r0 = part * (FH // 2)
        return _gelu2(_mm(w3_t[r0:r0 + FH // 2, :], _upk(n_w[n]))).astype(BF)

    def out_rows(n):
        if isinstance(n, int) and n == LAST_TILE:
            return ((0, RS), (RS, D))
        return ((0, D),)

    def m4(n, h3a, h3b):
        h3 = jnp.concatenate([h3a, h3b], axis=0)
        for r0, r1 in out_rows(n):
            w4 = jnp.concatenate([w4_w[j, r0 // 2:r1 // 2, :]
                                  for j in range(F // L)], axis=1)
            o_v[n, r0:r1, :] = (r_s[n, r0:r1, :] + 0.5 * _mm(w4, h3)).astype(BF)
            ocopy(n, r0, r1).start()

    def step(cfg, a=None, b=None, bw=None, c1=None, c23=None):
        order, ahead, seq = cfg
        ta, tb, tbw, tc1, tc23 = (None if v is None else _tiles(v)
                                  for v in (a, b, bw, c1, c23))
        xn, h3, toks = {}, {}, []
        for item in order.split():
            name, j = item[:-1], int(item[-1])
            if name in ("q", "k", "v"):
                if j not in xn:
                    xn[j] = ln1(ta[j])
                {"q": mq, "k": mk, "v": mv}[name](ta[j], xn[j])
            elif name == "o":
                mo(tb[j], attn(tb[j], toks, ahead, seq))
            elif name == "w1_":
                m1(tbw[j])
            elif name == "w2_":
                m2(tc1[j], j)
            elif name in ("w3a", "w3b"):
                h3[name, j] = m3(tc23[j], int(name == "w3b"))
            elif name == "w4_":
                m4(tc23[j], h3["w3a", j], h3["w3b", j])
            else:
                raise ValueError(item)

    def prep_wo():
        w32 = wo_n[...].astype(F32)
        for j in range(4):
            cw = min(L, D - j * L)
            wo32[j, :, 0:cw] = w32[:, j * L:j * L + cw]
        rows = []
        for dp in range(DH // 2):
            for half in range(2):
                for par in range(2):
                    r0 = half * 8 * DH + 2 * dp + par
                    rows.append(jnp.concatenate(
                        [wo32[j, pl.ds(r0, 8, stride=DH), 0:min(L, D - j * L)]
                         for j in range(4)], axis=1))
        wo_t[...] = _pk(jnp.concatenate(rows, axis=0).astype(BF).T)

    def prep(name):
        if name == "wo":
            prep_wo()
        elif name[0] == "c":
            i = int(name[1])
            wqkv_t[QC[i] // 2:QC[i + 1] // 2, :] = _pk(
                wqkv_n[:, QC[i]:QC[i + 1]].T)
        else:
            src, dst = {"w1": (w1_n, w1_t), "w2": (w2_n, w2_t),
                        "w3": (w3_n, w3_t)}[name]
            dst[...] = _pk(src[...].T)

    xn, pr, att, toks, ahead = {}, {}, {}, [], None
    for item in PROLOGUE.split():
        kind, _, arg = item.partition(":")
        if kind == "W":
            for name in arg.split("+"):
                for c in dma[name]:
                    c.wait()
            toks = []
        elif kind == "S":
            for c in dma[arg]:
                c.start(priority=1)
        elif kind == "T":
            prep(arg)
        elif kind == "A":
            ahead = int(arg) or None
        else:
            n = int(arg)
            if kind in ("l", "ql", "qh", "q", "k", "v") and n not in xn:
                xn[n] = ln1(n)
            if kind == "ql":
                mq(n, xn[n], 0, QC[1])
            elif kind == "qh":
                mq(n, xn[n], QC[1], D)
            elif kind in ("q", "k", "v"):
                {"q": mq, "k": mk, "v": mv}[kind](n, xn[n])
            elif kind == "aK":
                pr[n] = [probs(n, h, toks, ahead) for h in range(2)]
            elif kind == "aV":
                att[n] = interleave([mix(n, h, pr[n][h], toks, ahead)
                                     for h in range(2)])
            elif kind == "a":
                att[n] = attn(n, toks, ahead, "KVKV")
            elif kind == "o":
                mo(n, att[n])
            elif kind == "w1":
                m1(n)
            elif kind == "w2":
                m2(n, n % TB)
            elif kind != "l":
                raise ValueError(item)

    def steady(s, carry):
        u = s * TB
        step(CFG_S, a=_Idx(u, 4), b=_Idx(u, 3), bw=_Idx(u, 2), c1=_Idx(u, 1),
             c23=_Idx(u, 0))
        return carry + s

    total = lax.fori_loop(0, NB - 4, steady, 0)

    step(CFG_E, b=NB - 1, bw=NB - 2, c1=NB - 3, c23=NB - 4)

    @pl.when(total > 0)
    def _():
        step(CFG_F, bw=NB - 1, c1=NB - 2, c23=NB - 3)
        step(CFG_T, c1=NB - 1, c23=NB - 2)
        step(CFG_L, c23=NB - 1)

    for n in range(NT):
        for r0, r1 in out_rows(n):
            ocopy(n, r0, r1).wait()


@jax.jit
def pallas_sequential_preLN__sliding_local_dilated__mixer_s_mlp__prompt_kernel(
    A_x: jax.Array,
    A_wqkv: jax.Array,
    A_wo: jax.Array,
    B_x: jax.Array,
    B_w1: jax.Array,
    B_w2: jax.Array,
    B_w3: jax.Array,
    B_w4: jax.Array,
):
    del B_x
    xt = A_x.reshape(S, D).T
    hbm = pl.BlockSpec(memory_space=pltpu.HBM)
    out = pl.pallas_call(
        _kernel,
        out_shape=jax.ShapeDtypeStruct((D, S), BF),
        in_specs=[hbm] * 7,
        out_specs=hbm,
        scratch_shapes=[
            pltpu.VMEM((NT, D, L), BF),
            pltpu.VMEM((NT, D, L), BF),
            pltpu.VMEM((D, 3 * D), BF),
            pltpu.VMEM((D, D), BF),
            pltpu.VMEM((D, D), BF),
            pltpu.VMEM((D, D), BF),
            pltpu.VMEM((D, F), BF),
            pltpu.VMEM((F // L, D, L), BF),
            pltpu.VMEM((3 * DW, D), U32),
            pltpu.VMEM((DW, D), U32),
            pltpu.VMEM((DW, D), U32),
            pltpu.VMEM((DW, D), U32),
            pltpu.VMEM((FH, D), U32),
            pltpu.VMEM((4, D, L), F32),
            pltpu.VMEM((NT, D, L), F32),
            pltpu.VMEM((NT + 1, D, L), BF),
            pltpu.VMEM((NT + 1, D, L), BF),
            pltpu.VMEM((NT, D, L), F32),
            pltpu.VMEM((NT, 16, L), F32),
            pltpu.VMEM((NT + 2, D, L), BF),
            pltpu.VMEM((NT, D, L), BF),
            pltpu.VMEM((NT, D, L), F32),
            pltpu.VMEM((TB, D, L), F32),
            pltpu.VMEM((NT, D, L), BF),
            pltpu.SemaphoreType.DMA((len(_WAITS),)),
            pltpu.SemaphoreType.DMA((1,)),
        ],
        compiler_params=pltpu.CompilerParams(
            vmem_limit_bytes=64 * 1024 * 1024),
    )(xt, A_wqkv, A_wo, B_w1, B_w2, B_w3, B_w4.T)
    return out.T.reshape(1, S, D)
```
